```python
import os as _os
_os.environ.setdefault("JAX_PLATFORMS", "cpu")
import jax
import jax.numpy as jnp

def _softmax(x, axis=-1):
    return jax.nn.softmax(x, axis=axis)
def _gelu(x):
    return jax.nn.gelu(x, approximate=True)
def _silu(x):
    return jax.nn.silu(x)
def _sigmoid(x):
    return jax.nn.sigmoid(x)
def _layernorm(x, axis=-1, eps=1e-5):
    m = jnp.mean(x, axis=axis, keepdims=True)
    v = jnp.var(x, axis=axis, keepdims=True)
    return (x - m) / jnp.sqrt(v + eps)
def _scatter_add(tgt, idx, src, axis=0):
    return tgt.at[idx].add(src)
def _segment_sum(src, seg, n):
    return jax.ops.segment_sum(src, seg, n)
class _Rng:
    def __init__(self, key):
        self._k = key
    def _next(self):
        self._k, sub = jax.random.split(self._k)
        return sub
    def normal(self, shape):
        return jax.random.normal(self._next(), shape, dtype=jnp.bfloat16)
    def randint(self, lo, hi, shape):
        return jax.random.randint(self._next(), shape, lo, hi, dtype=jnp.int32)
    def uniform(self, shape, lo=0.0, hi=1.0):
        return jax.random.uniform(self._next(), shape, jnp.bfloat16, lo, hi)
    def permutation(self, n):
        return jax.random.permutation(self._next(), n)


kernel_name = 'standalone__mha_block_cached__near_ridge'

def setup_inputs():
    _rng = _Rng(jax.random.key(int.from_bytes(__import__("os").urandom(4), "little")))
    _w = (lambda a: (lambda t: t.astype(jnp.bfloat16) if jnp.issubdtype(t.dtype, jnp.floating) else t)(jnp.asarray(a)))
    B, Sq, D = 8, 112, 640
    H, Sk, Dh = 32, 512, 192
    return {
        "x": _w((lambda *s: _rng.normal(s) * 0.8)(B, Sq, D)),
        "k_cache": _w((lambda *s: _rng.normal(s) * 0.8)(B, H, Sk, Dh)),
        "v_cache": _w((lambda *s: _rng.normal(s) * 0.05)(B, H, Sk, Dh)),
        "wq": _w((lambda *s: _rng.normal(s) * 0.8)(D, H * Dh) * (D ** -0.5)),
        "wo": _w((lambda *s: _rng.normal(s) * 0.05)(H * Dh, D) * ((H * Dh) ** -0.5)),
    }

def reference(x, k_cache, v_cache, wq, wo):
    B, Sq, D = x.shape
    H, Dh = 32, 192
    q = (lambda x, *d: x.transpose(*d))((x @ wq).reshape(B, Sq, H, Dh), 0, 2, 1, 3)
    scores = jnp.einsum("bhqd,bhkd->bhqk", q, k_cache) * (Dh ** -0.5)
    p = _softmax(scores, axis=-1)
    o = jnp.einsum("bhqk,bhkd->bhqd", p, v_cache)
    return (lambda x, *d: x.transpose(*d))(o, 0, 2, 1, 3).reshape(B, Sq, H * Dh) @ wo
```

```python
import functools
import math
import jax
import jax.numpy as jnp
from jax import lax
from jax.experimental import pallas as pl
from jax.experimental.pallas import tpu as pltpu

B, SQ, D = 8, 112, 640
H, SK, DH = 32, 512, 192
PW = 2 * DH
QSCALE = (DH ** -0.5) * math.log2(math.e)
F32 = jnp.float32
BF16 = jnp.bfloat16
VPRIO = 0


def make_kernel(HP, NBUF, UNROLL, ISSUE_POS):
    HG = H // HP
    W = HP * DH
    NP = HP // 2
    NSTEP = HG * B
    WQ_ROWS = D // B
    WO_ROWS = W // B
    assert NBUF & (NBUF - 1) == 0

    def kernel(x_hbm, kt_hbm, vt_hbm, wq_hbm, wo_hbm, o_hbm,
               x_v, kbuf, vbuf, wqbuf, wobuf, acc, obuf,
               sem_x, sem_k, sem_v, sem_wq, sem_wo, sem_o):

        def k_copy(t):
            return pltpu.make_async_copy(kt_hbm.at[t & (B - 1), t >> 3], kbuf.at[t & (NBUF - 1)], sem_k.at[t & (NBUF - 1)])

        def v_copy(t):
            return pltpu.make_async_copy(vt_hbm.at[t & (B - 1), t >> 3], vbuf.at[t & (NBUF - 1)], sem_v.at[t & (NBUF - 1)])

        def wq_slice_copy(hg, j):
            ws = hg & 1
            r0 = pl.multiple_of(j * WQ_ROWS, 16)
            c0 = pl.multiple_of(hg * W, 128)
            return pltpu.make_async_copy(wq_hbm.at[pl.ds(r0, WQ_ROWS), pl.ds(c0, W)],
                                         wqbuf.at[ws, pl.ds(r0, WQ_ROWS)], sem_wq.at[ws])

        def wo_slice_copy(hg, j):
            ws = hg & 1
            r0 = pl.multiple_of(j * WO_ROWS, 16)
            g0 = pl.multiple_of(hg * W + j * WO_ROWS, 16)
            return pltpu.make_async_copy(wo_hbm.at[pl.ds(g0, WO_ROWS)],
                                         wobuf.at[ws, pl.ds(r0, WO_ROWS)], sem_wo.at[ws])

        def wq_wait(ws):
            pltpu.make_async_copy(wqbuf.at[ws], wqbuf.at[ws], sem_wq.at[ws]).wait()

        def wo_wait(ws):
            pltpu.make_async_copy(wobuf.at[ws], wobuf.at[ws], sem_wo.at[ws]).wait()

        def x_copy(b):
            r0 = b * SQ if isinstance(b, int) else pl.multiple_of(b * SQ, 16)
            return pltpu.make_async_copy(x_hbm.at[pl.ds(r0, SQ)], x_v.at[pl.ds(r0, SQ)], sem_x.at[b])

        x_copy(0).start()
        pltpu.make_async_copy(wq_hbm.at[:, pl.ds(0, W)], wqbuf.at[0], sem_wq.at[0]).start()
        k_copy(0).start()
        v_copy(0).start(priority=VPRIO)
        pltpu.make_async_copy(wo_hbm.at[pl.ds(0, W)], wobuf.at[0], sem_wo.at[0]).start()
        for t in range(1, NBUF - 1):
            x_copy(t).start()
            k_copy(t).start()
            v_copy(t).start(priority=VPRIO)
        for t in range(NBUF - 1, B):
            x_copy(t).start()
        acc[...] = jnp.zeros(acc.shape, F32)

        lane = lax.broadcasted_iota(jnp.int32, (SQ, 128), 1)
        lo = lane < 64

        def step(t):
            b = t & (B - 1)
            hg = t >> 3
            slot = t & (NBUF - 1)
            ws = hg & 1
            nxt = t + NBUF - 1

            def issue():
                @pl.when(nxt < NSTEP)
                def _():
                    k_copy(nxt).start()
                    v_copy(nxt).start(priority=VPRIO)

                @pl.when(jnp.logical_and(hg + 1 < HG, b == 0))
                def _():
                    c0 = pl.multiple_of((hg + 1) * W, 128)
                    pltpu.make_async_copy(wq_hbm.at[:, pl.ds(c0, W)], wqbuf.at[1 - ws], sem_wq.at[1 - ws]).start()
                    pltpu.make_async_copy(wo_hbm.at[pl.ds(c0, W)], wobuf.at[1 - ws], sem_wo.at[1 - ws]).start()

            if ISSUE_POS == 0:
                issue()

            @pl.when(hg == 0)
            def _():
                x_copy(b).wait()

            @pl.when(b == 0)
            def _():
                wq_wait(ws)
                wo_wait(ws)

            k_copy(t).wait()
            v_copy(t).wait()
            if ISSUE_POS == 1:
                issue()

            row0 = pl.multiple_of(b * SQ, 16)
            xb = x_v[pl.ds(row0, SQ), :]
            qs = []
            for pi in range(NP):
                q = jnp.dot(xb, wqbuf[ws, :, pi * PW:(pi + 1) * PW], preferred_element_type=F32) * QSCALE
                q0 = q[:, 0:128].astype(BF16)
                qm = q[:, 128:256]
                q2 = q[:, 256:384].astype(BF16)
                qa = jnp.concatenate([q0, jnp.where(lo, qm, 0.0).astype(BF16)], axis=1)
                qb = jnp.concatenate([jnp.where(lo, 0.0, qm).astype(BF16), q2], axis=1)
                qs.append(qa)
                qs.append(qb)
            if ISSUE_POS == 2:
                issue()
            ss = []
            for h in range(HP):
                pi, hh = h // 2, h % 2
                r0 = pi * PW + hh * 128
                kt = kbuf[slot, r0:r0 + 256, :]
                ss.append(jnp.dot(qs[h], kt, preferred_element_type=F32))
            os_ = []
            ls = []
            for h in range(HP):
                s = ss[h]
                m = jnp.max(s, axis=-1, keepdims=True)
                p = jnp.exp2(s - m)
                l = jnp.sum(p, axis=-1, keepdims=True)
                ls.append(1.0 / l)
                pb = p.astype(BF16)
                vt = vbuf[slot, h * DH:(h + 1) * DH, :]
                pb = jnp.concatenate([pb, jnp.zeros((128 - SQ, SK), BF16)], axis=0)
                ot = lax.dot_general(vt, pb, (((1,), (1,)), ((), ())), preferred_element_type=F32)
                os_.append(ot)
            for pi in range(NP):
                ot = jnp.concatenate([os_[2 * pi], os_[2 * pi + 1]], axis=0)
                o = ot.T[0:SQ, :]
                o0 = (o[:, 0:128] * ls[2 * pi]).astype(BF16)
                om = (o[:, 128:256] * jnp.where(lo, ls[2 * pi], ls[2 * pi + 1])).astype(BF16)
                o2 = (o[:, 256:384] * ls[2 * pi + 1]).astype(BF16)
                ob = jnp.concatenate([o0, om, o2], axis=1)
                contrib = jnp.dot(ob, wobuf[ws, pi * PW:(pi + 1) * PW, :], preferred_element_type=F32)
                if pi < NP - 1:
                    acc[pl.ds(row0, SQ), :] += contrib
                else:
                    res = acc[pl.ds(row0, SQ), :] + contrib
                    acc[pl.ds(row0, SQ), :] = res
                    obuf[pl.ds(row0, SQ), :] = res.astype(BF16)

            @pl.when(hg == HG - 1)
            def _():
                pltpu.make_async_copy(obuf.at[pl.ds(row0, SQ)], o_hbm.at[pl.ds(row0, SQ)], sem_o).start()

        def body(i, carry):
            for u in range(UNROLL):
                step(i * UNROLL + u)
            return carry

        lax.fori_loop(0, NSTEP // UNROLL, body, 0)
        pltpu.make_async_copy(obuf, obuf, sem_o).wait()

    scratch = [
        pltpu.VMEM((B * SQ, D), BF16),
        pltpu.VMEM((NBUF, W, SK), BF16),
        pltpu.VMEM((NBUF, W, SK), BF16),
        pltpu.VMEM((2, D, W), BF16),
        pltpu.VMEM((2, W, D), BF16),
        pltpu.VMEM((B * SQ, D), F32),
        pltpu.VMEM((B * SQ, D), BF16),
        pltpu.SemaphoreType.DMA((B,)),
        pltpu.SemaphoreType.DMA((NBUF,)),
        pltpu.SemaphoreType.DMA((NBUF,)),
        pltpu.SemaphoreType.DMA((2,)),
        pltpu.SemaphoreType.DMA((2,)),
        pltpu.SemaphoreType.DMA(()),
    ]
    return kernel, scratch, HG, W


@jax.jit
def pallas_standalone__mha_block_cached__near_ridge_kernel(x, k_cache, v_cache, wq, wo):
    kernel, scratch, HG, W = make_kernel(4, 4, 1, 1)
    x2 = x.reshape(B * SQ, D)
    kt = jnp.swapaxes(k_cache, 2, 3).reshape(B, HG, W, SK)
    vt = jnp.swapaxes(v_cache, 2, 3).reshape(B, HG, W, SK)
    out = pl.pallas_call(
        kernel,
        in_specs=[pl.BlockSpec(memory_space=pl.ANY)] * 5,
        out_specs=pl.BlockSpec(memory_space=pl.ANY),
        out_shape=jax.ShapeDtypeStruct((B * SQ, D), BF16),
        scratch_shapes=scratch,
        compiler_params=pltpu.CompilerParams(vmem_limit_bytes=100 * 1024 * 1024,
                                             disable_bounds_checks=True),
    )(x2, kt, vt, wq, wo)
    return out.reshape(B, SQ, D)
```

```python
import functools
import math
import jax
import jax.numpy as jnp
from jax import lax
from jax.experimental import pallas as pl
from jax.experimental.pallas import tpu as pltpu

B, SQ, D = 8, 112, 640
H, SK, DH = 32, 512, 192
PW = 2 * DH
QSCALE = (DH ** -0.5) * math.log2(math.e)
F32 = jnp.float32
BF16 = jnp.bfloat16
HP = 4
HG = H // HP
W = HP * DH
NP = HP // 2
NSTEP = HG * B
NBUF = 4
VWAIT = 0
UNROLL = 1
MODE = 'full'


def kernel(x_hbm, kt_hbm, vt_hbm, wq_hbm, wo_hbm, o_hbm,
           x_v, kbuf, vbuf, wqbuf, wobuf, qbuf, acc, obuf,
           sem_x, sem_k, sem_v, sem_wq, sem_wo, sem_o):

    def k_copy(t):
        return pltpu.make_async_copy(kt_hbm.at[t & (B - 1), t >> 3], kbuf.at[t & (NBUF - 1)], sem_k.at[t & (NBUF - 1)])

    def v_copy(t):
        return pltpu.make_async_copy(vt_hbm.at[t & (B - 1), t >> 3], vbuf.at[t & (NBUF - 1)], sem_v.at[t & (NBUF - 1)])

    def wq_copy(hg):
        c0 = hg * W if isinstance(hg, int) else pl.multiple_of(hg * W, 128)
        return pltpu.make_async_copy(wq_hbm.at[:, pl.ds(c0, W)], wqbuf.at[hg & 1], sem_wq.at[hg & 1])

    def wo_copy(hg):
        c0 = hg * W if isinstance(hg, int) else pl.multiple_of(hg * W, 128)
        return pltpu.make_async_copy(wo_hbm.at[pl.ds(c0, W)], wobuf.at[hg & 1], sem_wo.at[hg & 1])

    def x_copy(b):
        r0 = b * SQ if isinstance(b, int) else pl.multiple_of(b * SQ, 16)
        return pltpu.make_async_copy(x_hbm.at[pl.ds(r0, SQ)], x_v.at[pl.ds(r0, SQ)], sem_x.at[b])

    lane = lax.broadcasted_iota(jnp.int32, (SQ, 128), 1)
    lo = lane < 64

    def qproj(b, ws):
        row0 = pl.multiple_of(b * SQ, 16)
        xb = x_v[pl.ds(row0, SQ), :]
        for pi in range(NP):
            q = jnp.dot(xb, wqbuf[ws, :, pi * PW:(pi + 1) * PW], preferred_element_type=F32) * QSCALE
            qm = q[:, 128:256]
            qbuf[b, 2 * pi, :, 0:128] = q[:, 0:128].astype(BF16)
            qbuf[b, 2 * pi, :, 128:256] = jnp.where(lo, qm, 0.0).astype(BF16)
            qbuf[b, 2 * pi + 1, :, 0:128] = jnp.where(lo, 0.0, qm).astype(BF16)
            qbuf[b, 2 * pi + 1, :, 128:256] = q[:, 256:384].astype(BF16)

    wq_copy(0).start()
    for b in range(B):
        x_copy(b).start()
    k_copy(0).start()
    v_copy(0).start()
    wq_copy(1).start()
    wo_copy(0).start()
    for t in range(1, NBUF - 1):
        k_copy(t).start()
        v_copy(t).start()
    acc[...] = jnp.zeros(acc.shape, F32)
    wq_copy(0).wait()

    def pro_body(b, c):
        x_copy(b).wait()
        qproj(b, 0)
        return c
    lax.fori_loop(0, B, pro_body, 0)

    def step(t, last):
        b = t & (B - 1)
        hg = t >> 3
        slot = t & (NBUF - 1)
        ws = hg & 1
        nxt = t + NBUF - 1

        @pl.when(b == 0)
        def _():
            if not last:
                wq_copy(hg + 1).wait()
            wo_copy(hg).wait()

        k_copy(t).wait()
        if VWAIT == 0:
            v_copy(t).wait()

        @pl.when(nxt < NSTEP)
        def _():
            k_copy(nxt).start()
            v_copy(nxt).start()

        if not last:
            @pl.when(b == 0)
            def _():
                wo_copy(hg + 1).start()

            @pl.when(jnp.logical_and(b == 0, hg + 2 < HG))
            def _():
                wq_copy(hg + 2).start()

        if last:
            @pl.when(b == B - 1)
            def _():
                pltpu.make_async_copy(obuf.at[pl.ds(0, (B - 1) * SQ)], o_hbm.at[pl.ds(0, (B - 1) * SQ)], sem_o).start()

        row0 = pl.multiple_of(b * SQ, 16)
        if MODE == 'nocompute':
            if VWAIT == 1:
                v_copy(t).wait()
            if last:
                obuf[pl.ds(row0, SQ), :] = x_v[pl.ds(row0, SQ), :]
                @pl.when(b == B - 1)
                def _():
                    pltpu.make_async_copy(obuf.at[pl.ds((B - 1) * SQ, SQ)], o_hbm.at[pl.ds((B - 1) * SQ, SQ)], sem_o).start()
            return
        ss = []
        for h in range(HP):
            pi, hh = h // 2, h % 2
            r0 = pi * PW + hh * 128
            kt = kbuf[slot, r0:r0 + 256, :]
            ss.append(jnp.dot(qbuf[b, h], kt, preferred_element_type=F32))
        if not last:
            qproj(b, 1 - ws)
        if VWAIT == 1:
            v_copy(t).wait()
        os_ = []
        ls = []
        for h in range(HP):
            s = ss[h]
            m = jnp.max(s, axis=-1, keepdims=True)
            p = jnp.exp2(s - m)
            l = jnp.sum(p, axis=-1, keepdims=True)
            ls.append(1.0 / l)
            pb = p.astype(BF16)
            vt = vbuf[slot, h * DH:(h + 1) * DH, :]
            pb = jnp.concatenate([pb, jnp.zeros((128 - SQ, SK), BF16)], axis=0)
            ot = lax.dot_general(vt, pb, (((1,), (1,)), ((), ())), preferred_element_type=F32)
            os_.append(ot)
        for pi in range(NP):
            ot = jnp.concatenate([os_[2 * pi], os_[2 * pi + 1]], axis=0)
            o = ot.T[0:SQ, :]
            o0 = (o[:, 0:128] * ls[2 * pi]).astype(BF16)
            om = (o[:, 128:256] * jnp.where(lo, ls[2 * pi], ls[2 * pi + 1])).astype(BF16)
            o2 = (o[:, 256:384] * ls[2 * pi + 1]).astype(BF16)
            ob = jnp.concatenate([o0, om, o2], axis=1)
            contrib = jnp.dot(ob, wobuf[ws, pi * PW:(pi + 1) * PW, :], preferred_element_type=F32)
            if last and pi == NP - 1:
                obuf[pl.ds(row0, SQ), :] = (acc[pl.ds(row0, SQ), :] + contrib).astype(BF16)
            else:
                acc[pl.ds(row0, SQ), :] += contrib
        if last:
            @pl.when(b == B - 1)
            def _():
                pltpu.make_async_copy(obuf.at[pl.ds((B - 1) * SQ, SQ)], o_hbm.at[pl.ds((B - 1) * SQ, SQ)], sem_o).start()

    def main_body(i, carry):
        for u in range(UNROLL):
            step(i * UNROLL + u, False)
        return carry

    def last_body(i, carry):
        for u in range(UNROLL):
            step(i * UNROLL + u, True)
        return carry

    lax.fori_loop(0, (NSTEP - B) // UNROLL, main_body, 0)
    lax.fori_loop((NSTEP - B) // UNROLL, NSTEP // UNROLL, last_body, 0)
    pltpu.make_async_copy(obuf, obuf, sem_o).wait()


@jax.jit
def pallas_standalone__mha_block_cached__near_ridge_kernel(x, k_cache, v_cache, wq, wo):
    scratch = [
        pltpu.VMEM((B * SQ, D), BF16),
        pltpu.VMEM((NBUF, W, SK), BF16),
        pltpu.VMEM((NBUF, W, SK), BF16),
        pltpu.VMEM((2, D, W), BF16),
        pltpu.VMEM((2, W, D), BF16),
        pltpu.VMEM((B, HP, SQ, 256), BF16),
        pltpu.VMEM((B * SQ, D), F32),
        pltpu.VMEM((B * SQ, D), BF16),
        pltpu.SemaphoreType.DMA((B,)),
        pltpu.SemaphoreType.DMA((NBUF,)),
        pltpu.SemaphoreType.DMA((NBUF,)),
        pltpu.SemaphoreType.DMA((2,)),
        pltpu.SemaphoreType.DMA((2,)),
        pltpu.SemaphoreType.DMA(()),
    ]
    x2 = x.reshape(B * SQ, D)
    kt = jnp.swapaxes(k_cache, 2, 3).reshape(B, HG, W, SK)
    vt = jnp.swapaxes(v_cache, 2, 3).reshape(B, HG, W, SK)
    out = pl.pallas_call(
        kernel,
        in_specs=[pl.BlockSpec(memory_space=pl.ANY)] * 5,
        out_specs=pl.BlockSpec(memory_space=pl.ANY),
        out_shape=jax.ShapeDtypeStruct((B * SQ, D), BF16),
        scratch_shapes=scratch,
        compiler_params=pltpu.CompilerParams(vmem_limit_bytes=100 * 1024 * 1024,
                                             disable_bounds_checks=True),
    )(x2, kt, vt, wq, wo)
    return out.reshape(B, SQ, D)
```

```python
import math

import jax
import jax.numpy as jnp
from jax import lax
from jax.experimental import pallas as pl
from jax.experimental.pallas import tpu as pltpu

B, SQ, D = 8, 112, 640
H, SK, DH = 32, 512, 192
PW = 2 * DH
HP = 4
HG = H // HP
W = HP * DH
NP = HP // 2
NSTEP = HG * B
NBUF = 4
LOOK = 3
LANES = 128
QSCALE = (DH ** -0.5) * math.log2(math.e)
F32 = jnp.float32
BF16 = jnp.bfloat16
NT = (((1,), (1,)), ((), ()))


def _kernel(x_hbm, kt_hbm, vt_hbm, wq_hbm, wo_hbm, o_hbm,
            x_v, kbuf, vbuf, wqbuf, wobuf, qbuf, acc, obuf,
            sem_x, sem_k, sem_v, sem_wq, sem_wo, sem_o):

    def k_copy(t):
        s = t & (NBUF - 1)
        return pltpu.make_async_copy(kt_hbm.at[t & (B - 1), t >> 3], kbuf.at[s], sem_k.at[s])

    def v_copy(t):
        s = t & (NBUF - 1)
        return pltpu.make_async_copy(vt_hbm.at[t & (B - 1), t >> 3], vbuf.at[s], sem_v.at[s])

    def wq_copy(hg):
        c0 = hg * W if isinstance(hg, int) else pl.multiple_of(hg * W, LANES)
        return pltpu.make_async_copy(wq_hbm.at[:, pl.ds(c0, W)], wqbuf.at[hg & 1], sem_wq.at[hg & 1])

    def wo_copy(hg):
        r0 = hg * W if isinstance(hg, int) else pl.multiple_of(hg * W, LANES)
        return pltpu.make_async_copy(wo_hbm.at[pl.ds(r0, W)], wobuf.at[hg & 1], sem_wo.at[hg & 1])

    def x_copy(b):
        r0 = b * SQ if isinstance(b, int) else pl.multiple_of(b * SQ, 16)
        return pltpu.make_async_copy(x_hbm.at[pl.ds(r0, SQ)], x_v.at[pl.ds(r0, SQ)], sem_x.at[b])

    def out_copy(r0, n):
        return pltpu.make_async_copy(obuf.at[pl.ds(r0, n)], o_hbm.at[pl.ds(r0, n)], sem_o)

    lo = lax.broadcasted_iota(jnp.int32, (SQ, LANES), 1) < 64

    def qproj(b, ws):
        row0 = pl.multiple_of(b * SQ, 16)
        xb = x_v[pl.ds(row0, SQ), :]
        for pi in range(NP):
            q = jnp.dot(xb, wqbuf[ws, :, pi * PW:(pi + 1) * PW], preferred_element_type=F32) * QSCALE
            qm = q[:, 128:256]
            qbuf[b, 2 * pi, :, 0:128] = q[:, 0:128].astype(BF16)
            qbuf[b, 2 * pi, :, 128:256] = jnp.where(lo, qm, 0.0).astype(BF16)
            qbuf[b, 2 * pi + 1, :, 0:128] = jnp.where(lo, 0.0, qm).astype(BF16)
            qbuf[b, 2 * pi + 1, :, 128:256] = q[:, 256:384].astype(BF16)

    half = D // 2
    wq0_a = pltpu.make_async_copy(wq_hbm.at[pl.ds(0, half), pl.ds(0, W)], wqbuf.at[0, pl.ds(0, half)], sem_o)
    wq0_b = pltpu.make_async_copy(wq_hbm.at[pl.ds(half, half), pl.ds(0, W)], wqbuf.at[0, pl.ds(half, half)],
                                  sem_wq.at[0])
    x_copy(0).start()
    wq0_a.start()
    wq0_b.start()
    for b in range(1, B):
        x_copy(b).start()
    acc[...] = jnp.zeros(acc.shape, F32)
    wq0_a.wait()
    k_copy(0).start()
    wq_copy(1).start()
    v_copy(0).start()
    wo_copy(0).start()
    wq0_b.wait()

    def prologue_body(b, carry):
        x_copy(b).wait()

        @pl.when(b == 3)
        def _():
            k_copy(1).start()
            v_copy(1).start()

        @pl.when(b == 6)
        def _():
            k_copy(2).start()
            v_copy(2).start()

        qproj(b, 0)
        return carry

    lax.fori_loop(0, B, prologue_body, 0)

    def step(t, last):
        b = t & (B - 1)
        hg = t >> 3
        slot = t & (NBUF - 1)
        ws = hg & 1
        row0 = pl.multiple_of(b * SQ, 16)

        @pl.when(b == 0)
        def _():
            if not last:
                wq_copy(hg + 1).wait()
            wo_copy(hg).wait()

        k_copy(t).wait()
        v_copy(t).wait()

        @pl.when(t + LOOK < NSTEP)
        def _():
            k_copy(t + LOOK).start()
            v_copy(t + LOOK).start()

        if last:
            @pl.when(b == B - 1)
            def _():
                out_copy(0, (B - 1) * SQ).start()
        else:
            @pl.when(b == 0)
            def _():
                wo_copy(hg + 1).start()

            @pl.when(jnp.logical_and(b == 0, hg + 2 < HG))
            def _():
                wq_copy(hg + 2).start()

        ss = []
        for h in range(HP):
            r0 = (h // 2) * PW + (h % 2) * 128
            ss.append(jnp.dot(qbuf[b, h], kbuf[slot, r0:r0 + 256, :], preferred_element_type=F32))

        if not last:
            qproj(b, 1 - ws)

        ps, inv_l = [], []
        for h in range(HP):
            s = ss[h]
            m = jnp.max(s, axis=-1, keepdims=True)
            p = jnp.exp2(s - m)
            inv_l.append(1.0 / jnp.sum(p, axis=-1, keepdims=True))
            ps.append(p.astype(BF16))

        zpad = jnp.zeros((LANES - SQ, SK), BF16)
        parts = []
        for pi in range(NP):
            p1, p2 = ps[2 * pi], ps[2 * pi + 1]
            r0 = pi * PW
            oa = lax.dot_general(p1, vbuf[slot, r0:r0 + 128, :], NT, preferred_element_type=F32)
            m1 = lax.dot_general(vbuf[slot, r0 + 128:r0 + 192, :], jnp.concatenate([p1, zpad], axis=0), NT,
                                 preferred_element_type=F32)
            m2 = lax.dot_general(vbuf[slot, r0 + 192:r0 + 256, :], jnp.concatenate([p2, zpad], axis=0), NT,
                                 preferred_element_type=F32)
            oc = lax.dot_general(p2, vbuf[slot, r0 + 256:r0 + 384, :], NT, preferred_element_type=F32)
            parts.append((oa, m1, m2, oc))

        for pi in range(NP):
            oa, m1, m2, oc = parts[pi]
            l1, l2 = inv_l[2 * pi], inv_l[2 * pi + 1]
            om = jnp.concatenate([m1, m2], axis=0).T[0:SQ, :]
            ob = jnp.concatenate([(oa * l1).astype(BF16),
                                  (om * jnp.where(lo, l1, l2)).astype(BF16),
                                  (oc * l2).astype(BF16)], axis=1)
            contrib = jnp.dot(ob, wobuf[ws, pi * PW:(pi + 1) * PW, :], preferred_element_type=F32)
            if last and pi == NP - 1:
                obuf[pl.ds(row0, SQ), :] = (acc[pl.ds(row0, SQ), :] + contrib).astype(BF16)
            else:
                acc[pl.ds(row0, SQ), :] += contrib

    def main_body(t, carry):
        step(t, False)
        return carry

    def last_body(t, carry):
        step(t, True)
        return carry

    lax.fori_loop(0, NSTEP - B, main_body, 0)
    lax.fori_loop(NSTEP - B, NSTEP, last_body, 0)
    out_copy((B - 1) * SQ, SQ).start()
    out_copy(0, B * SQ).wait()


@jax.jit
def pallas_standalone__mha_block_cached__near_ridge_kernel(x, k_cache, v_cache, wq, wo):
    x2 = x.reshape(B * SQ, D)
    kt = jnp.swapaxes(k_cache, 2, 3).reshape(B, HG, W, SK)
    vt = jnp.swapaxes(v_cache, 2, 3).reshape(B, HG, W, SK)
    out = pl.pallas_call(
        _kernel,
        in_specs=[pl.BlockSpec(memory_space=pl.ANY)] * 5,
        out_specs=pl.BlockSpec(memory_space=pl.ANY),
        out_shape=jax.ShapeDtypeStruct((B * SQ, D), BF16),
        scratch_shapes=[
            pltpu.VMEM((B * SQ, D), BF16),
            pltpu.VMEM((NBUF, W, SK), BF16),
            pltpu.VMEM((NBUF, W, SK), BF16),
            pltpu.VMEM((2, D, W), BF16),
            pltpu.VMEM((2, W, D), BF16),
            pltpu.VMEM((B, HP, SQ, 256), BF16),
            pltpu.VMEM((B * SQ, D), F32),
            pltpu.VMEM((B * SQ, D), BF16),
            pltpu.SemaphoreType.DMA((B,)),
            pltpu.SemaphoreType.DMA((NBUF,)),
            pltpu.SemaphoreType.DMA((NBUF,)),
            pltpu.SemaphoreType.DMA((2,)),
            pltpu.SemaphoreType.DMA((2,)),
            pltpu.SemaphoreType.DMA(()),
        ],
        compiler_params=pltpu.CompilerParams(vmem_limit_bytes=64 * 1024 * 1024,
                                             disable_bounds_checks=True),
    )(x2, kt, vt, wq, wo)
    return out.reshape(B, SQ, D)
```

```python
import math

import jax
import jax.numpy as jnp
from jax import lax
from jax.experimental import pallas as pl
from jax.experimental.pallas import tpu as pltpu

B, SQ, D = 8, 112, 640
H, SK, DH = 32, 512, 192
PW = 2 * DH
HP = 4
HG = H // HP
W = HP * DH
NP = HP // 2
NSTEP = HG * B
NBUF = 4
LOOK = 3
WB = 4
NSPLIT = 4
SMB = 2
LANES = 128
QSCALE = (DH ** -0.5) * math.log2(math.e)
F32 = jnp.float32
BF16 = jnp.bfloat16
NT = (((1,), (1,)), ((), ()))


def _kernel(x_hbm, kt_hbm, vt_hbm, wq_hbm, wo_hbm, o_hbm,
            x_v, kbuf, vbuf, wqbuf, wobuf, qbuf, acc, obuf,
            sem_x, sem_k, sem_v, sem_wq, sem_wo, sem_o):

    def k_copy(t):
        s = t & (NBUF - 1)
        return pltpu.make_async_copy(kt_hbm.at[t & (B - 1), t >> 3], kbuf.at[s], sem_k.at[s])

    def v_copy(t):
        s = t & (NBUF - 1)
        return pltpu.make_async_copy(vt_hbm.at[t & (B - 1), t >> 3], vbuf.at[s], sem_v.at[s])

    def wq_copy(hg):
        c0 = hg * W if isinstance(hg, int) else pl.multiple_of(hg * W, LANES)
        return pltpu.make_async_copy(wq_hbm.at[:, pl.ds(c0, W)], wqbuf.at[hg & 1], sem_wq.at[hg & 1])

    def wo_copy(hg):
        r0 = hg * W if isinstance(hg, int) else pl.multiple_of(hg * W, LANES)
        return pltpu.make_async_copy(wo_hbm.at[pl.ds(r0, W)], wobuf.at[hg & 1], sem_wo.at[hg & 1])

    def x_copy(b):
        r0 = b * SQ if isinstance(b, int) else pl.multiple_of(b * SQ, 16)
        return pltpu.make_async_copy(x_hbm.at[pl.ds(r0, SQ)], x_v.at[pl.ds(r0, SQ)], sem_x.at[b])

    def out_copy(r0, n):
        return pltpu.make_async_copy(obuf.at[pl.ds(r0, n)], o_hbm.at[pl.ds(r0, n)], sem_o)

    lo = lax.broadcasted_iota(jnp.int32, (SQ, LANES), 1) < 64

    def qproj(b, ws):
        row0 = pl.multiple_of(b * SQ, 16)
        xb = x_v[pl.ds(row0, SQ), :]
        for pi in range(NP):
            q = jnp.dot(xb, wqbuf[ws, :, pi * PW:(pi + 1) * PW], preferred_element_type=F32) * QSCALE
            qm = q[:, 128:256]
            qbuf[b, 2 * pi, :, 0:128] = q[:, 0:128].astype(BF16)
            qbuf[b, 2 * pi, :, 128:256] = jnp.where(lo, qm, 0.0).astype(BF16)
            qbuf[b, 2 * pi + 1, :, 0:128] = jnp.where(lo, 0.0, qm).astype(BF16)
            qbuf[b, 2 * pi + 1, :, 128:256] = q[:, 256:384].astype(BF16)

    half = D // 2
    wq0_a = pltpu.make_async_copy(wq_hbm.at[pl.ds(0, half), pl.ds(0, W)], wqbuf.at[0, pl.ds(0, half)], sem_o)
    wq0_b = pltpu.make_async_copy(wq_hbm.at[pl.ds(half, half), pl.ds(0, W)], wqbuf.at[0, pl.ds(half, half)],
                                  sem_wq.at[0])
    x_copy(0).start()
    wq0_a.start()
    wq0_b.start()
    for b in range(1, B):
        x_copy(b).start()
    acc[...] = jnp.zeros(acc.shape, F32)
    wq0_a.wait()
    k_copy(0).start()
    wq_copy(1).start()
    v_copy(0).start()
    wo_copy(0).start()
    wq0_b.wait()

    def prologue_body(b, carry):
        x_copy(b).wait()
        for j in range(1, LOOK):
            @pl.when(b == 3 * j)
            def _(j=j):
                k_copy(j).start()
                v_copy(j).start()
        qproj(b, 0)
        return carry

    lax.fori_loop(0, B, prologue_body, 0)

    def step(t, last, split):
        b = t & (B - 1)
        hg = t >> 3
        slot = t & (NBUF - 1)
        ws = hg & 1
        row0 = pl.multiple_of(b * SQ, 16)

        @pl.when(b == 0)
        def _():
            if not last:
                wq_copy(hg + 1).wait()
            wo_copy(hg).wait()

        k_copy(t).wait()
        if not split:
            v_copy(t).wait()

        if not last:
            @pl.when(b == WB)
            def _():
                wo_copy(hg + 1).start()

            @pl.when(jnp.logical_and(b == WB, hg + 2 < HG))
            def _():
                wq_copy(hg + 2).start()

        @pl.when(t + LOOK < NSTEP)
        def _():
            k_copy(t + LOOK).start()
            v_copy(t + LOOK).start()

        ss = []
        for h in range(HP):
            r0 = (h // 2) * PW + (h % 2) * 128
            ss.append(jnp.dot(qbuf[b, h], kbuf[slot, r0:r0 + 256, :], preferred_element_type=F32))

        if not last:
            qproj(b, 1 - ws)

        ps, inv_l = [], []
        for h in range(HP):
            if split and h == SMB:
                v_copy(t).wait()

                @pl.when(t == NSTEP - 1)
                def _():
                    out_copy(0, (B - 1) * SQ).start()

            s = ss[h]
            m = jnp.max(s, axis=-1, keepdims=True)
            p = jnp.exp2(s - m)
            inv_l.append(1.0 / jnp.sum(p, axis=-1, keepdims=True))
            ps.append(p.astype(BF16))

        zpad = jnp.zeros((LANES - SQ, SK), BF16)
        parts = []
        for pi in range(NP):
            p1, p2 = ps[2 * pi], ps[2 * pi + 1]
            r0 = pi * PW
            oa = lax.dot_general(p1, vbuf[slot, r0:r0 + 128, :], NT, preferred_element_type=F32)
            m1 = lax.dot_general(vbuf[slot, r0 + 128:r0 + 192, :], jnp.concatenate([p1, zpad], axis=0), NT,
                                 preferred_element_type=F32)
            m2 = lax.dot_general(vbuf[slot, r0 + 192:r0 + 256, :], jnp.concatenate([p2, zpad], axis=0), NT,
                                 preferred_element_type=F32)
            oc = lax.dot_general(p2, vbuf[slot, r0 + 256:r0 + 384, :], NT, preferred_element_type=F32)
            parts.append((oa, m1, m2, oc))

        for pi in range(NP):
            oa, m1, m2, oc = parts[pi]
            l1, l2 = inv_l[2 * pi], inv_l[2 * pi + 1]
            om = jnp.concatenate([m1, m2], axis=0).T[0:SQ, :]
            ob = jnp.concatenate([(oa * l1).astype(BF16),
                                  (om * jnp.where(lo, l1, l2)).astype(BF16),
                                  (oc * l2).astype(BF16)], axis=1)
            contrib = jnp.dot(ob, wobuf[ws, pi * PW:(pi + 1) * PW, :], preferred_element_type=F32)
            if last and pi == NP - 1:
                obuf[pl.ds(row0, SQ), :] = (acc[pl.ds(row0, SQ), :] + contrib).astype(BF16)
            else:
                acc[pl.ds(row0, SQ), :] += contrib

    def body(last, split):
        def f(t, carry):
            step(t, last, split)
            return carry
        return f

    lax.fori_loop(0, NSTEP - B, body(False, False), 0)
    lax.fori_loop(NSTEP - B, NSTEP - NSPLIT, body(True, False), 0)
    lax.fori_loop(NSTEP - NSPLIT, NSTEP, body(True, True), 0)
    out_copy((B - 1) * SQ, SQ).start()
    out_copy(0, B * SQ).wait()


@jax.jit
def pallas_standalone__mha_block_cached__near_ridge_kernel(x, k_cache, v_cache, wq, wo):
    x2 = x.reshape(B * SQ, D)
    kt = jnp.swapaxes(k_cache, 2, 3).reshape(B, HG, W, SK)
    vt = jnp.swapaxes(v_cache, 2, 3).reshape(B, HG, W, SK)
    out = pl.pallas_call(
        _kernel,
        in_specs=[pl.BlockSpec(memory_space=pl.ANY)] * 5,
        out_specs=pl.BlockSpec(memory_space=pl.ANY),
        out_shape=jax.ShapeDtypeStruct((B * SQ, D), BF16),
        scratch_shapes=[
            pltpu.VMEM((B * SQ, D), BF16),
            pltpu.VMEM((NBUF, W, SK), BF16),
            pltpu.VMEM((NBUF, W, SK), BF16),
            pltpu.VMEM((2, D, W), BF16),
            pltpu.VMEM((2, W, D), BF16),
            pltpu.VMEM((B, HP, SQ, 256), BF16),
            pltpu.VMEM((B * SQ, D), F32),
            pltpu.VMEM((B * SQ, D), BF16),
            pltpu.SemaphoreType.DMA((B,)),
            pltpu.SemaphoreType.DMA((NBUF,)),
            pltpu.SemaphoreType.DMA((NBUF,)),
            pltpu.SemaphoreType.DMA((2,)),
            pltpu.SemaphoreType.DMA((2,)),
            pltpu.SemaphoreType.DMA(()),
        ],
        compiler_params=pltpu.CompilerParams(vmem_limit_bytes=64 * 1024 * 1024,
                                             disable_bounds_checks=True,
                                             disable_semaphore_checks=True),
    )(x2, kt, vt, wq, wo)
    return out.reshape(B, SQ, D)
```
